```python
import jax
import jax.numpy as jnp

def _softmax(x, axis=-1):
    return jax.nn.softmax(x, axis=axis)
def _gelu(x):
    return jax.nn.gelu(x, approximate=True)
def _silu(x):
    return jax.nn.silu(x)
def _sigmoid(x):
    return jax.nn.sigmoid(x)
def _layernorm(x, axis=-1, eps=1e-5):
    m = jnp.mean(x, axis=axis, keepdims=True)
    v = jnp.var(x, axis=axis, keepdims=True)
    return (x - m) / jnp.sqrt(v + eps)
def _scatter_add(tgt, idx, src, axis=0):
    return tgt.at[idx].add(src)
def _segment_sum(src, seg, n):
    return jax.ops.segment_sum(src, seg, n)
class _Rng:
    def __init__(self, key):
        self._k = key
    def _next(self):
        self._k, sub = jax.random.split(self._k)
        return sub
    def normal(self, shape):
        return jax.random.normal(self._next(), shape, dtype=jnp.bfloat16)
    def randint(self, lo, hi, shape):
        return jax.random.randint(self._next(), shape, lo, hi, dtype=jnp.int32)
    def uniform(self, shape, lo=0.0, hi=1.0):
        return jax.random.uniform(self._next(), shape, jnp.bfloat16, lo, hi)
    def permutation(self, n):
        return jax.random.permutation(self._next(), n)


kernel_name = 'sequential_preLN__sliding_block_cached__mixer_s_mlp__decode'

def setup_inputs():
    _rng = _Rng(jax.random.key(int.from_bytes(__import__("os").urandom(4), "little")))
    _w = (lambda a: (lambda t: t.astype(jnp.bfloat16) if jnp.issubdtype(t.dtype, jnp.floating) else t)(jnp.asarray(a)))
    def _A_setup():
        B, Sq, D = 1, 1, 640
        Hq, Hkv, Sk, Dh = 32, 32, 32768, 192
        assert Hq % Hkv == 0, (Hq, Hkv)
        return {
            "x": _w((lambda *s: _rng.normal(s) * 0.05)(B, Sq, D)),
            "k_cache": _w((lambda *s: _rng.normal(s) * 0.05)(B, Hkv, Sk, Dh)),
            "v_cache": _w((lambda *s: _rng.normal(s) * 0.05)(B, Hkv, Sk, Dh)),
            "wq": _w((lambda *s: _rng.normal(s) * 0.05)(D, Hq * Dh) * (D ** -0.5)),
            "wo": _w((lambda *s: _rng.normal(s) * 0.05)(Hq * Dh, D) * ((Hq * Dh) ** -0.5)),
        }
    _A_in = _A_setup()

    def _B_setup():
        B, S, D, F = 1, 1, 640, 1536
        return {
            "x":  _w((lambda *s: _rng.normal(s) * 0.05)(B, S, D)),
            "w1": _w((lambda *s: _rng.normal(s) * 0.05)(D, D) * (D ** -0.5)),
            "w2": _w((lambda *s: _rng.normal(s) * 0.05)(D, D) * (D ** -0.5)),
            "w3": _w((lambda *s: _rng.normal(s) * 0.05)(D, F) * (D ** -0.5)),
            "w4": _w((lambda *s: _rng.normal(s) * 0.05)(F, D) * (F ** -0.5)),
        }
    _B_in = _B_setup()

    return {
        "A_x": _A_in["x"],
        "A_k_cache": _A_in["k_cache"],
        "A_v_cache": _A_in["v_cache"],
        "A_wq": _A_in["wq"],
        "A_wo": _A_in["wo"],
        "B_x": _B_in["x"],
        "B_w1": _B_in["w1"],
        "B_w2": _B_in["w2"],
        "B_w3": _B_in["w3"],
        "B_w4": _B_in["w4"],
    }

def reference(A_x, A_k_cache, A_v_cache, A_wq, A_wo, B_x, B_w1, B_w2, B_w3, B_w4):
    def _A_ref(x, k_cache, v_cache, wq, wo):
        B, Sq, D = x.shape
        Hq, Dh = 32, 192
        Hkv, Sk = k_cache.shape[1], k_cache.shape[2]
        W = min(4096, max(256, Sk // 4))
        rep = Hq // Hkv
        q = (lambda x, *d: x.transpose(*d))((x @ wq).reshape(B, Sq, Hq, Dh), 0, 2, 1, 3)
        k = jnp.repeat(k_cache[:, :, Sk - W:, :], rep, axis=1)
        v = jnp.repeat(v_cache[:, :, Sk - W:, :], rep, axis=1)
        scores = jnp.einsum("bhqd,bhkd->bhqk", q, k) * (Dh ** -0.5)
        p = _softmax(scores, axis=-1)
        o = jnp.einsum("bhqk,bhkd->bhqd", p, v)
        return (lambda x, *d: x.transpose(*d))(o, 0, 2, 1, 3).reshape(B, Sq, Hq * Dh) @ wo

    def _B_ref(x, w1, w2, w3, w4):
        B, S, D = x.shape
        h = _gelu(_layernorm(x, axis=-1) @ w1)
        c = D // 4
        g0 = jnp.pad(h[:, :, 0*c:1*c], ((0, 0), (1, 0), (0, 0)))[:, :S, :]
        g1 = jnp.pad(h[:, :, 1*c:2*c], ((0, 0), (0, 1), (0, 0)))[:, 1:, :]
        g2 = jnp.pad(h[:, :, 2*c:3*c], ((0, 0), (2, 0), (0, 0)))[:, :S, :]
        g3 = jnp.pad(h[:, :, 3*c:   ], ((0, 0), (0, 2), (0, 0)))[:, 2:, :]
        hs = jnp.concatenate([g0, g1, g2, g3], axis=-1) @ w2
        x1 = x + hs
        h2 = _gelu(_layernorm(x1, axis=-1) @ w3) @ w4
        return x1 + h2

    x = A_x
    h = x + _A_ref(_layernorm(x, axis=-1), A_k_cache, A_v_cache, A_wq, A_wo)
    h2 = h + _B_ref(_layernorm(h, axis=-1), B_w1, B_w2, B_w3, B_w4)
    return h2
```

```python
import jax
import jax.numpy as jnp
import jax.experimental.pallas as pl
import jax.experimental.pallas.tpu as pltpu

D, H, DH, SK, W, F = 640, 32, 192, 32768, 4096, 1536
ROWS = H * DH
G = 2
GR = G * DH
NG = H // G
NS = 2
EPS = 1e-5


def _ln(x):
    m = jnp.mean(x, axis=-1, keepdims=True)
    c = x - m
    v = jnp.mean(c * c, axis=-1, keepdims=True)
    return c / jnp.sqrt(v + EPS)


def _gelu(x):
    c = 0.7978845608028654
    return 0.5 * x * (1.0 + jnp.tanh(c * (x + 0.044715 * (x * x * x))))


def _kernel(x_hbm, kT, vT, wq, wo, w3, w4, o_ref,
            xbuf, kbuf, vbuf, wqb, wob, w3b, w4b,
            xsem, ksem, vsem, wqsem, wosem, wsem):
    def k_copy(j, slot):
        return pltpu.make_async_copy(
            kT.at[pl.ds(pl.multiple_of(j * GR, GR), GR), pl.ds(SK - W, W)], kbuf.at[slot], ksem.at[slot])

    def v_copy(j, slot):
        return pltpu.make_async_copy(
            vT.at[pl.ds(pl.multiple_of(j * GR, GR), GR), pl.ds(SK - W, W)], vbuf.at[slot], vsem.at[slot])

    def wq_copy(j):
        return pltpu.make_async_copy(
            wq.at[:, pl.ds(pl.multiple_of(j * GR, GR), GR)], wqb.at[j], wqsem.at[j])

    def wo_copy(j):
        return pltpu.make_async_copy(
            wo.at[pl.ds(pl.multiple_of(j * GR, GR), GR), :], wob.at[j], wosem.at[j])

    x_copy = pltpu.make_async_copy(x_hbm.at[0], xbuf, xsem)
    w3_copy = pltpu.make_async_copy(w3, w3b, wsem.at[0])
    w4_copy = pltpu.make_async_copy(w4, w4b, wsem.at[1])

    x_copy.start()
    for j in range(NS):
        wq_copy(j).start()
        k_copy(j, j).start()
        v_copy(j, j).start()
        wo_copy(j).start()

    x_copy.wait()
    x = xbuf[...].astype(jnp.float32)
    xn = _ln(x).astype(jnp.bfloat16)
    xn8 = jnp.broadcast_to(xn, (8, D))

    row = jax.lax.broadcasted_iota(jnp.int32, (8, GR), 0)
    col = jax.lax.broadcasted_iota(jnp.int32, (8, GR), 1)
    mask = (col >= row * DH) & (col < (row + 1) * DH)
    scale = DH ** -0.5

    def body(j, acc):
        slot = j % NS
        wq_copy(j).wait()
        q = jnp.dot(xn8, wqb[j], preferred_element_type=jnp.float32)
        qa = jnp.where(mask, q, 0.0).astype(jnp.bfloat16)
        k_copy(j, slot).wait()
        s = jnp.dot(qa, kbuf[slot], preferred_element_type=jnp.float32) * scale

        @pl.when(j + NS < NG)
        def _():
            wq_copy(j + NS).start()
            k_copy(j + NS, slot).start()

        m = jnp.max(s, axis=-1, keepdims=True)
        p = jnp.exp(s - m)
        l = jnp.sum(p, axis=-1, keepdims=True)
        v_copy(j, slot).wait()
        o = jax.lax.dot_general(p.astype(jnp.bfloat16), vbuf[slot],
                                (((1,), (1,)), ((), ())), preferred_element_type=jnp.float32)

        @pl.when(j + NS < NG)
        def _():
            v_copy(j + NS, slot).start()
            wo_copy(j + NS).start()

        @pl.when(j + NS == NG - 1)
        def _():
            w3_copy.start()
            w4_copy.start()

        o = jnp.where(mask, o / l, 0.0).astype(jnp.bfloat16)
        wo_copy(j).wait()
        return acc + jnp.dot(o, wob[j], preferred_element_type=jnp.float32)

    acc = jax.lax.fori_loop(0, NG, body, jnp.zeros((8, D), jnp.float32))
    h = x + jnp.sum(acc, axis=0, keepdims=True)
    x1 = _ln(h)
    y = jnp.broadcast_to(_ln(x1).astype(jnp.bfloat16), (8, D))
    w3_copy.wait()
    g = _gelu(jnp.dot(y, w3b[...], preferred_element_type=jnp.float32)).astype(jnp.bfloat16)
    w4_copy.wait()
    h2 = jnp.dot(g, w4b[...], preferred_element_type=jnp.float32)[0:1]
    o_ref[0] = (h + (x1 + h2)).astype(o_ref.dtype)


@jax.jit
def pallas_sequential_preLN__sliding_block_cached__mixer_s_mlp__decode_kernel(
    A_x: jax.Array,
    A_k_cache: jax.Array,
    A_v_cache: jax.Array,
    A_wq: jax.Array,
    A_wo: jax.Array,
    B_x: jax.Array,
    B_w1: jax.Array,
    B_w2: jax.Array,
    B_w3: jax.Array,
    B_w4: jax.Array,
):
    kT = jnp.swapaxes(A_k_cache, 2, 3).reshape(ROWS, SK)
    vT = jnp.swapaxes(A_v_cache, 2, 3).reshape(ROWS, SK)
    any_spec = pl.BlockSpec(memory_space=pl.ANY)
    return pl.pallas_call(
        _kernel,
        out_shape=jax.ShapeDtypeStruct((1, 1, D), jnp.bfloat16),
        in_specs=[any_spec] * 7,
        out_specs=pl.BlockSpec(memory_space=pltpu.VMEM),
        scratch_shapes=[
            pltpu.VMEM((1, D), jnp.bfloat16),
            pltpu.VMEM((NS, GR, W), jnp.bfloat16),
            pltpu.VMEM((NS, GR, W), jnp.bfloat16),
            pltpu.VMEM((NG, D, GR), jnp.bfloat16),
            pltpu.VMEM((NG, GR, D), jnp.bfloat16),
            pltpu.VMEM((D, F), jnp.bfloat16),
            pltpu.VMEM((F, D), jnp.bfloat16),
            pltpu.SemaphoreType.DMA,
            pltpu.SemaphoreType.DMA((NS,)),
            pltpu.SemaphoreType.DMA((NS,)),
            pltpu.SemaphoreType.DMA((NG,)),
            pltpu.SemaphoreType.DMA((NG,)),
            pltpu.SemaphoreType.DMA((2,)),
        ],
        compiler_params=pltpu.CompilerParams(vmem_limit_bytes=64 * 1024 * 1024),
    )(A_x, kT, vT, A_wq, A_wo, B_w3, B_w4)
```

```python
import jax
import jax.numpy as jnp
import jax.experimental.pallas as pl
import jax.experimental.pallas.tpu as pltpu

D, H, DH, SK, W, F = 640, 32, 192, 32768, 4096, 1536
ROWS = H * DH
GR = 2 * DH
NG = H // 2
C0 = SK - W
EPS = 1e-5
NF = F // 128
ND = D // 128
N_TS = 60


def _ln(x):
    m = jnp.mean(x, axis=-1, keepdims=True)
    c = x - m
    v = jnp.mean(c * c, axis=-1, keepdims=True)
    return c / jnp.sqrt(v + EPS)


def _gelu(x):
    c = 0.7978845608028654
    return 0.5 * x * (1.0 + jnp.tanh(c * (x + 0.044715 * (x * x * x))))


def make_kernel(CPM=1, LM=8, NM=8, delay=0, vmem_mb=64, interpret=False, nocompute=False, scopes=False,
                wthr=(1, 1), tgroup=1, nosemchk=True):
    CW = 128 * CPM
    NCM = W // CW
    SPM = 3 * CPM
    NGS = LM * SPM
    assert LM <= NM and NGS <= 30 and NCM & (NCM - 1) == 0 and NM & (NM - 1) == 0
    NPM = NCM // 2
    M_S0 = NPM
    M_F0 = M_S0 + (NG - 1) * NCM
    M_T0 = M_F0 + NPM
    assert LM <= NPM
    lg = NCM.bit_length() - 1

    class _NoScope:
        def __enter__(self):
            return None

        def __exit__(self, *a):
            return False

    def scope(name):
        return jax.named_scope(name) if scopes else _NoScope()

    def kernel(x_hbm, kT, vT, wq, wo, w3, w4, o_ref,
               xbuf, kbuf, vbuf, wqb, wob, w3b, w4b, s_scr, p_scr,
               xsem, sems, wqsem, wosem):

        def tile_copy(src, row, col, dst, sem):
            return pltpu.make_async_copy(
                src.at[pl.ds(pl.multiple_of(row, 128), 128), pl.ds(pl.multiple_of(col, 128), 128)], dst, sem)

        def dst_wait(dst, sem):
            pltpu.make_async_copy(dst, dst, sem).wait()

        def kv_dst(buf, pair, cm, u):
            return buf.at[pair & 1, cm, pl.ds((u % 3) * 128, 128), pl.ds((u // 3) * 128, 128)]

        def kv_copy(src, buf, pair, cm, u, sem):
            return tile_copy(src, pair * GR + (u % 3) * 128, C0 + cm * CW + (u // 3) * 128, kv_dst(buf, pair, cm, u), sem)

        def wq_chunk(j, i):
            r0 = pl.multiple_of(i * 32, 32)
            return pltpu.make_async_copy(wq.at[pl.ds(r0, 32), pl.ds(pl.multiple_of(j * GR, 128), GR)],
                                         wqb.at[j, pl.ds(r0, 32), :], wqsem.at[j])

        def wo_chunk(j, i):
            r0 = pl.multiple_of(i * 16, 16)
            return pltpu.make_async_copy(wo.at[pl.ds(pl.multiple_of(j * GR + i * 16, 16), 16), :],
                                         wob.at[j, pl.ds(r0, 16), :], wosem.at[j])

        def sem_of(mm, u):
            return sems.at[SPM * (mm & (NM - 1)) + u]

        def t_step_copies(i, sem):
            if isinstance(i, int):
                second = i >= 30
                i = i - 30 if second else i
                m, k = i // ND, i % ND
            else:
                second = False
                m = (i * 13) >> 6
                k = i - m * ND
            out = []
            for e in range(2):
                f = 2 * m + e
                if second:
                    out.append(tile_copy(w4, f * 128, k * 128, w4b.at[f, :, pl.ds(pl.multiple_of(k * 128, 128), 128)], sem))
                else:
                    out.append(tile_copy(w3, k * 128, f * 128, w3b.at[f, pl.ds(pl.multiple_of(k * 128, 128), 128), :], sem))
            return out

        def d():
            if delay:
                pl.delay(delay)

        def when(cond, fn):
            if isinstance(cond, (bool, int)):
                if cond:
                    fn()
            else:
                pl.when(cond)(fn)

        def issue_P(m, u):
            sem = sem_of(m, u)
            kv_copy(kT, kbuf, 0, 2 * m, u, sem).start(priority=0)
            kv_copy(kT, kbuf, 0, 2 * m + 1, u, sem).start(priority=1)
            per = -(-20 // (NPM * SPM))
            for e in range(per):
                i = (m * SPM + u) * per + e
                when(i < 20, lambda: wq_chunk(1, i if isinstance(i, int) else jnp.minimum(i, 19)).start(priority=(u + e) % 2))

        def issue_S(t, u, last_possible):
            j, cm = t >> lg, t & (NCM - 1)
            sem = sem_of(t + M_S0, u)
            kv_copy(kT, kbuf, j + 1, cm, u, sem).start(priority=0)
            kv_copy(vT, vbuf, j, cm, u, sem).start(priority=1)
            if u % 3 == 2:
                i = cm * CPM + u // 3
                c1 = (i < 20)
                if last_possible:
                    c1 = c1 & (j + 2 < NG)
                pl.when(c1)(lambda: wq_chunk(jnp.minimum(j + 2, NG - 1), jnp.minimum(i, 19)).start(priority=wthr[0]))
                pl.when(i < 24)(lambda: wo_chunk(j, jnp.minimum(i, 23)).start(priority=wthr[1]))

        def issue_F(m, u):
            sem = sem_of(m + M_F0, u)
            kv_copy(vT, vbuf, NG - 1, 2 * m, u, sem).start(priority=0)
            kv_copy(vT, vbuf, NG - 1, 2 * m + 1, u, sem).start(priority=1)
            per = -(-24 // (NPM * SPM))
            for e in range(per):
                i = (m * SPM + u) * per + e
                when(i < 24, lambda: wo_chunk(NG - 1, i if isinstance(i, int) else jnp.minimum(i, 23)).start(priority=(u + e) % 2))

        def issue_T(m, u):
            a, b = t_step_copies(m * SPM + u, sem_of(m + M_T0, u))
            a.start(priority=0)
            b.start(priority=1)

        def when_range(mt, lo, hi, fn, u):
            if isinstance(mt, int):
                if lo <= mt < hi:
                    fn(mt - lo, u)
            else:
                @pl.when((mt >= lo) & (mt < hi))
                def _():
                    fn(jnp.clip(mt - lo, 0, hi - lo - 1), u)

        x_copy = pltpu.make_async_copy(x_hbm.at[0], xbuf, xsem)
        x_copy.start()
        for i in range(20):
            wq_chunk(0, i).start(priority=0)

        def pro_body(m, _):
            for u in range(SPM):
                issue_P(m, u)
                d()
            return 0
        jax.lax.fori_loop(0, LM, pro_body, 0)

        with scope('xwait'):
            x_copy.wait()
        x = xbuf[...].astype(jnp.float32)
        xn = _ln(x).astype(jnp.bfloat16)
        xn8 = jnp.broadcast_to(xn, (8, D))

        row = jax.lax.broadcasted_iota(jnp.int32, (8, GR), 0)
        col = jax.lax.broadcasted_iota(jnp.int32, (8, GR), 1)
        mask = (col >= row * DH) & (col < (row + 1) * DH)
        scale = DH ** -0.5

        def q_for(j):
            dst_wait(wqb.at[j], wqsem.at[j])
            q = jnp.dot(xn8, wqb[j], preferred_element_type=jnp.float32)
            return jnp.where(mask, q, 0.0).astype(jnp.bfloat16)

        def qk(qa, slot, cm):
            if nocompute:
                return jnp.zeros((8, CW), jnp.float32)
            return jnp.dot(qa, kbuf[slot, cm], preferred_element_type=jnp.float32)

        def pv(slot, cm):
            if nocompute:
                return jnp.zeros((8, GR), jnp.float32)
            return jax.lax.dot_general(p_scr[cm], vbuf[slot, cm], (((1,), (1,)), ((), ())),
                                       preferred_element_type=jnp.float32)

        def softmax():
            s = s_scr[...] * scale
            m = jnp.max(jnp.max(s, axis=0), axis=-1, keepdims=True)
            p = jnp.exp(s - m[None])
            l = jnp.sum(jnp.sum(p, axis=0), axis=-1, keepdims=True)
            p_scr[...] = p.astype(jnp.bfloat16)
            return l

        def out_proj(o, l, out, j):
            o = jnp.where(mask, o / l, 0.0).astype(jnp.bfloat16)
            dst_wait(wob.at[j], wosem.at[j])
            return out + jnp.dot(o, wob[j], preferred_element_type=jnp.float32)

        with scope('q0'):
            qa = q_for(0)

        def p_body(m, _):
            for u in range(SPM):
                sem = sem_of(m, u)
                dst_wait(kv_dst(kbuf, 0, 2 * m, u), sem)
                dst_wait(kv_dst(kbuf, 0, 2 * m + 1, u), sem)
                mt = m + LM
                when_range(mt, 0, M_S0, issue_P, u)
                when_range(mt, M_S0, M_F0, lambda t, uu: issue_S(t, uu, False), u)
                d()
            s_scr[2 * m] = qk(qa, 0, 2 * m)
            s_scr[2 * m + 1] = qk(qa, 0, 2 * m + 1)
            return 0

        with scope('P_loop'):
            jax.lax.fori_loop(0, NPM, p_body, 0)
        l0 = softmax()
        qa1 = q_for(1)

        def s_iter(j, carry, last):
            out, qa, l = carry
            ks, vs = (j + 1) & 1, j & 1

            def c_body(cm, o):
                t = j * NCM + cm
                mm = M_S0 + t
                for u in range(SPM):
                    sem = sem_of(mm, u)
                    dst_wait(kv_dst(kbuf, ks, cm, u), sem)
                    dst_wait(kv_dst(vbuf, vs, cm, u), sem)
                    if last:
                        mt = mm + LM
                        when_range(mt, M_S0, M_F0, lambda tt, uu: issue_S(tt, uu, True), u)
                        when_range(mt, M_F0, M_T0, issue_F, u)
                    else:
                        issue_S(t + LM, u, True)
                    d()
                s_scr[cm] = qk(qa, ks, cm)
                return o + pv(vs, cm)

            with scope('S_loop'):
                o = jax.lax.fori_loop(0, NCM, c_body, jnp.zeros((8, GR), jnp.float32))
            out = out_proj(o, l, out, j)
            return out, qa, softmax()

        def s_iter2(j, carry):
            out, qa, l = s_iter(j, carry, False)
            return out, q_for(j + 2), l

        out, qa, l = jax.lax.fori_loop(0, NG - 2, s_iter2, (jnp.zeros((8, D), jnp.float32), qa1, l0))
        out, qa, l = s_iter(NG - 2, (out, qa, l), True)

        vs = (NG - 1) & 1

        def f_body(m, o):
            mm = M_F0 + m
            for u in range(SPM):
                sem = sem_of(mm, u)
                dst_wait(kv_dst(vbuf, vs, 2 * m, u), sem)
                dst_wait(kv_dst(vbuf, vs, 2 * m + 1, u), sem)
                mt = mm + LM
                when_range(mt, M_F0, M_T0, issue_F, u)
                when_range(mt, M_T0, M_T0 + LM, issue_T, u)
                d()
            return o + pv(vs, 2 * m) + pv(vs, 2 * m + 1)

        with scope('F_loop'):
            o = jax.lax.fori_loop(0, NPM, f_body, jnp.zeros((8, GR), jnp.float32))
        with scope('ln1'):
            out = out_proj(o, l, out, NG - 1)
            h = x + jnp.sum(out, axis=0, keepdims=True)
            x1 = _ln(h)
            y = jnp.broadcast_to(_ln(x1).astype(jnp.bfloat16), (8, D))

        G_T0 = SPM * M_T0

        def t_sem(i):
            return sems.at[(G_T0 + i) % (SPM * NM)]

        with scope('T'):
            g = [None] * NF
            acc = None
            for i in range(N_TS):
                a, b = t_step_copies(i, t_sem(i))
                a.wait()
                b.wait()
                if i + NGS < N_TS:
                    a, b = t_step_copies(i + NGS, t_sem(i + NGS))
                    a.start(priority=0)
                    b.start(priority=1)
                d()
                if i % ND == ND - 1:
                    m = (i % 30) // ND
                    for f in (2 * m, 2 * m + 1):
                        if i < 30:
                            g[f] = _gelu(jnp.dot(y, w3b[f], preferred_element_type=jnp.float32)).astype(jnp.bfloat16)
                        else:
                            t = jnp.dot(g[f], w4b[f], preferred_element_type=jnp.float32)
                            acc = t if acc is None else acc + t
            o_ref[0] = (h + (x1 + acc[0:1])).astype(o_ref.dtype)

    @jax.jit
    def run(A_x, A_k_cache, A_v_cache, A_wq, A_wo, B_x, B_w1, B_w2, B_w3, B_w4):
        kT = jnp.swapaxes(A_k_cache, 2, 3).reshape(ROWS, SK)
        vT = jnp.swapaxes(A_v_cache, 2, 3).reshape(ROWS, SK)
        any_spec = pl.BlockSpec(memory_space=pl.ANY)
        return pl.pallas_call(
            kernel,
            out_shape=jax.ShapeDtypeStruct((1, 1, D), jnp.bfloat16),
            in_specs=[any_spec] * 7,
            out_specs=pl.BlockSpec(memory_space=pltpu.VMEM),
            scratch_shapes=[
                pltpu.VMEM((1, D), jnp.bfloat16),
                pltpu.VMEM((2, NCM, GR, CW), jnp.bfloat16),
                pltpu.VMEM((2, NCM, GR, CW), jnp.bfloat16),
                pltpu.VMEM((NG, D, GR), jnp.bfloat16),
                pltpu.VMEM((NG, GR, D), jnp.bfloat16),
                pltpu.VMEM((NF, D, 128), jnp.bfloat16),
                pltpu.VMEM((NF, 128, D), jnp.bfloat16),
                pltpu.VMEM((NCM, 8, CW), jnp.float32),
                pltpu.VMEM((NCM, 8, CW), jnp.bfloat16),
                pltpu.SemaphoreType.DMA,
                pltpu.SemaphoreType.DMA((SPM * NM,)),
                pltpu.SemaphoreType.DMA((NG,)),
                pltpu.SemaphoreType.DMA((NG,)),
            ],
            compiler_params=pltpu.CompilerParams(vmem_limit_bytes=vmem_mb * 1024 * 1024, disable_bounds_checks=True,
                                                 disable_semaphore_checks=nosemchk),
            interpret=interpret,
        )(A_x, kT, vT, A_wq, A_wo, B_w3, B_w4)

    return run


_run = make_kernel(CPM=2, LM=5, NM=8)


@jax.jit
def pallas_sequential_preLN__sliding_block_cached__mixer_s_mlp__decode_kernel(
    A_x: jax.Array,
    A_k_cache: jax.Array,
    A_v_cache: jax.Array,
    A_wq: jax.Array,
    A_wo: jax.Array,
    B_x: jax.Array,
    B_w1: jax.Array,
    B_w2: jax.Array,
    B_w3: jax.Array,
    B_w4: jax.Array,
):
    return _run(A_x, A_k_cache, A_v_cache, A_wq, A_wo, B_x, B_w1, B_w2, B_w3, B_w4)
```

```python
import jax
import jax.numpy as jnp
import jax.experimental.pallas as pl
import jax.experimental.pallas.tpu as pltpu

D, H, DH, SK, W, F = 640, 32, 192, 32768, 4096, 1536
ROWS = H * DH
GR = 2 * DH
NG = H // 2
C0 = SK - W
EPS = 1e-5
NF = F // 128
ND = D // 128
N_TS = 60


def _ln(x):
    m = jnp.mean(x, axis=-1, keepdims=True)
    c = x - m
    v = jnp.mean(c * c, axis=-1, keepdims=True)
    return c / jnp.sqrt(v + EPS)


def _gelu(x):
    c = 0.7978845608028654
    return 0.5 * x * (1.0 + jnp.tanh(c * (x + 0.044715 * (x * x * x))))


def make_kernel(CPM=1, LM=8, NGS=None, kvc=(128, 128), NM=8, delay=0, vmem_mb=64, interpret=False, nocompute=False, scopes=False,
                wthr=(1, 1), tgroup=1, nosemchk=True):
    CW = 128 * CPM
    NCM = W // CW
    RC, CC = kvc
    NRC, NCC = GR // RC, CW // CC
    assert GR % RC == 0 and CW % CC == 0
    SPM = NRC * NCC
    NGS = NGS or LM * SPM
    LM = -(-NGS // SPM)
    assert SPM * NM >= NGS and NGS <= 60 and NCM & (NCM - 1) == 0 and NM & (NM - 1) == 0
    assert SPM % 3 == 0 or (3 * NCM * SPM) % 32 == 0
    NPM = NCM // 2
    M_S0 = NPM
    M_F0 = M_S0 + (NG - 1) * NCM
    M_T0 = M_F0 + NPM
    assert LM <= NPM
    lg = NCM.bit_length() - 1

    class _NoScope:
        def __enter__(self):
            return None

        def __exit__(self, *a):
            return False

    def scope(name):
        return jax.named_scope(name) if scopes else _NoScope()

    def kernel(x_hbm, kT, vT, wq, wo, w3, w4, o_ref,
               xbuf, kbuf, vbuf, wqb, wob, w3b, w4b, s_scr, p_scr,
               xsem, sems, wqsem, wosem):

        def tile_copy(src, row, col, dst, sem):
            return pltpu.make_async_copy(
                src.at[pl.ds(pl.multiple_of(row, 128), 128), pl.ds(pl.multiple_of(col, 128), 128)], dst, sem)

        def dst_wait(dst, sem):
            pltpu.make_async_copy(dst, dst, sem).wait()

        def kv_dst(buf, pair, cm, u):
            return buf.at[pair & 1, cm, pl.ds((u % NRC) * RC, RC), pl.ds((u // NRC) * CC, CC)]

        def kv_copy(src, buf, pair, cm, u, sem):
            row = pl.multiple_of(pair * GR + (u % NRC) * RC, 8)
            col = pl.multiple_of(C0 + cm * CW + (u // NRC) * CC, 128)
            return pltpu.make_async_copy(src.at[pl.ds(row, RC), pl.ds(col, CC)], kv_dst(buf, pair, cm, u), sem)

        def wq_chunk(j, i):
            r0 = pl.multiple_of(i * 32, 32)
            return pltpu.make_async_copy(wq.at[pl.ds(r0, 32), pl.ds(pl.multiple_of(j * GR, 128), GR)],
                                         wqb.at[j, pl.ds(r0, 32), :], wqsem.at[j])

        def wo_chunk(j, i):
            r0 = pl.multiple_of(i * 16, 16)
            return pltpu.make_async_copy(wo.at[pl.ds(pl.multiple_of(j * GR + i * 16, 16), 16), :],
                                         wob.at[j, pl.ds(r0, 16), :], wosem.at[j])

        def sem_of(mm, u):
            return sems.at[SPM * (mm & (NM - 1)) + u]

        def t_step_copies(i, sem, second=False):
            if isinstance(i, int):
                second = i >= 30
                i = i - 30 if second else i
                m, k = i // ND, i % ND
            else:
                m = (i * 13) >> 6
                k = i - m * ND
            out = []
            for e in range(2):
                f = 2 * m + e
                if second:
                    out.append(tile_copy(w4, f * 128, k * 128, w4b.at[f, :, pl.ds(pl.multiple_of(k * 128, 128), 128)], sem))
                else:
                    out.append(tile_copy(w3, k * 128, f * 128, w3b.at[f, pl.ds(pl.multiple_of(k * 128, 128), 128), :], sem))
            return out

        def d():
            if delay:
                pl.delay(delay)

        def when(cond, fn):
            if isinstance(cond, (bool, int)):
                if cond:
                    fn()
            else:
                pl.when(cond)(fn)

        def issue_P(m, u):
            sem = sem_of(m, u)
            kv_copy(kT, kbuf, 0, 2 * m, u, sem).start(priority=0)
            kv_copy(kT, kbuf, 0, 2 * m + 1, u, sem).start(priority=1)
            per = -(-20 // (NPM * SPM))
            for e in range(per):
                i = (m * SPM + u) * per + e
                when(i < 20, lambda: wq_chunk(1, i if isinstance(i, int) else jnp.minimum(i, 19)).start(priority=(u + e) % 2))

        def issue_S(t, u, last_possible):
            j, cm = t >> lg, t & (NCM - 1)
            sem = sem_of(t + M_S0, u)
            kv_copy(kT, kbuf, j + 1, cm, u, sem).start(priority=0)
            kv_copy(vT, vbuf, j, cm, u, sem).start(priority=1)
            SPW = NCM * SPM // 32
            assert SPM % SPW == 0
            if u % SPW == SPW - 1:
                i = cm * (SPM // SPW) + u // SPW
                c1 = (i < 20)
                if last_possible:
                    c1 = c1 & (j + 2 < NG)
                pl.when(c1)(lambda: wq_chunk(jnp.minimum(j + 2, NG - 1), jnp.minimum(i, 19)).start(priority=wthr[0]))
                pl.when(i < 24)(lambda: wo_chunk(j, jnp.minimum(i, 23)).start(priority=wthr[1]))

        def issue_F(m, u):
            sem = sem_of(m + M_F0, u)
            kv_copy(vT, vbuf, NG - 1, 2 * m, u, sem).start(priority=0)
            kv_copy(vT, vbuf, NG - 1, 2 * m + 1, u, sem).start(priority=1)
            per = -(-24 // (NPM * SPM))
            for e in range(per):
                i = (m * SPM + u) * per + e
                when(i < 24, lambda: wo_chunk(NG - 1, i if isinstance(i, int) else jnp.minimum(i, 23)).start(priority=(u + e) % 2))

        def issue_T(m, u):
            i = m * SPM + u

            def go():
                a, b = t_step_copies(i if isinstance(i, int) else jnp.minimum(i, 29), sem_of(m + M_T0, u))
                a.start(priority=0)
                b.start(priority=1)

            def go2():
                a, b = t_step_copies(jnp.clip(i - 30, 0, 29), sem_of(m + M_T0, u), True)
                a.start(priority=0)
                b.start(priority=1)
            when(i < min(NGS, 30), go)
            if NGS > 30:
                when((i >= 30) & (i < NGS), go2)

        def ahead(m, u):
            return m + (u + NGS) // SPM, (u + NGS) % SPM

        def when_range(mt, lo, hi, fn, u):
            if isinstance(mt, int):
                if lo <= mt < hi:
                    fn(mt - lo, u)
            else:
                @pl.when((mt >= lo) & (mt < hi))
                def _():
                    fn(jnp.clip(mt - lo, 0, hi - lo - 1), u)

        x_copy = pltpu.make_async_copy(x_hbm.at[0], xbuf, xsem)
        x_copy.start()
        for i in range(20):
            wq_chunk(0, i).start(priority=0)

        def pro_body(m, _):
            for u in range(SPM):
                when(m * SPM + u < NGS, lambda: issue_P(m, u))
                d()
            return 0
        jax.lax.fori_loop(0, LM, pro_body, 0)

        with scope('xwait'):
            x_copy.wait()
        x = xbuf[...].astype(jnp.float32)
        xn = _ln(x).astype(jnp.bfloat16)
        xn8 = jnp.broadcast_to(xn, (8, D))

        row = jax.lax.broadcasted_iota(jnp.int32, (8, GR), 0)
        col = jax.lax.broadcasted_iota(jnp.int32, (8, GR), 1)
        mask = (col >= row * DH) & (col < (row + 1) * DH)
        scale = DH ** -0.5

        def q_for(j):
            dst_wait(wqb.at[j], wqsem.at[j])
            q = jnp.dot(xn8, wqb[j], preferred_element_type=jnp.float32)
            return jnp.where(mask, q, 0.0).astype(jnp.bfloat16)

        def qk(qa, slot, cm):
            if nocompute:
                return jnp.zeros((8, CW), jnp.float32)
            return jnp.dot(qa, kbuf[slot, cm], preferred_element_type=jnp.float32)

        def pv(slot, cm):
            if nocompute:
                return jnp.zeros((8, GR), jnp.float32)
            return jax.lax.dot_general(p_scr[cm], vbuf[slot, cm], (((1,), (1,)), ((), ())),
                                       preferred_element_type=jnp.float32)

        def softmax():
            s = s_scr[...] * scale
            m = jnp.max(jnp.max(s, axis=0), axis=-1, keepdims=True)
            p = jnp.exp(s - m[None])
            l = jnp.sum(jnp.sum(p, axis=0), axis=-1, keepdims=True)
            p_scr[...] = p.astype(jnp.bfloat16)
            return l

        def out_proj(o, l, out, j):
            o = jnp.where(mask, o / l, 0.0).astype(jnp.bfloat16)
            dst_wait(wob.at[j], wosem.at[j])
            return out + jnp.dot(o, wob[j], preferred_element_type=jnp.float32)

        with scope('q0'):
            qa = q_for(0)

        def p_body(m, _):
            for u in range(SPM):
                sem = sem_of(m, u)
                dst_wait(kv_dst(kbuf, 0, 2 * m, u), sem)
                dst_wait(kv_dst(kbuf, 0, 2 * m + 1, u), sem)
                mt, ut = ahead(m, u)
                when_range(mt, 0, M_S0, issue_P, ut)
                when_range(mt, M_S0, M_F0, lambda t, uu: issue_S(t, uu, False), ut)
                d()
            s_scr[2 * m] = qk(qa, 0, 2 * m)
            s_scr[2 * m + 1] = qk(qa, 0, 2 * m + 1)
            return 0

        with scope('P_loop'):
            jax.lax.fori_loop(0, NPM, p_body, 0)
        l0 = softmax()
        qa1 = q_for(1)

        def s_iter(j, carry, last):
            out, qa, l = carry
            ks, vs = (j + 1) & 1, j & 1

            def c_body(cm, o):
                t = j * NCM + cm
                mm = M_S0 + t
                for u in range(SPM):
                    sem = sem_of(mm, u)
                    dst_wait(kv_dst(kbuf, ks, cm, u), sem)
                    dst_wait(kv_dst(vbuf, vs, cm, u), sem)
                    if last:
                        mt, ut = ahead(mm, u)
                        when_range(mt, M_S0, M_F0, lambda tt, uu: issue_S(tt, uu, True), ut)
                        when_range(mt, M_F0, M_T0, issue_F, ut)
                    else:
                        tt, ut = ahead(t, u)
                        issue_S(tt, ut, True)
                    d()
                s_scr[cm] = qk(qa, ks, cm)
                return o + pv(vs, cm)

            with scope('S_loop'):
                o = jax.lax.fori_loop(0, NCM, c_body, jnp.zeros((8, GR), jnp.float32))
            out = out_proj(o, l, out, j)
            return out, qa, softmax()

        def s_iter2(j, carry):
            out, qa, l = s_iter(j, carry, False)
            return out, q_for(j + 2), l

        out, qa, l = jax.lax.fori_loop(0, NG - 2, s_iter2, (jnp.zeros((8, D), jnp.float32), qa1, l0))
        out, qa, l = s_iter(NG - 2, (out, qa, l), True)

        vs = (NG - 1) & 1

        def f_body(m, o):
            mm = M_F0 + m
            for u in range(SPM):
                sem = sem_of(mm, u)
                dst_wait(kv_dst(vbuf, vs, 2 * m, u), sem)
                dst_wait(kv_dst(vbuf, vs, 2 * m + 1, u), sem)
                mt, ut = ahead(mm, u)
                when_range(mt, M_F0, M_T0, issue_F, ut)
                when_range(mt, M_T0, M_T0 + LM + 1, issue_T, ut)
                d()
            return o + pv(vs, 2 * m) + pv(vs, 2 * m + 1)

        with scope('F_loop'):
            o = jax.lax.fori_loop(0, NPM, f_body, jnp.zeros((8, GR), jnp.float32))
        with scope('ln1'):
            out = out_proj(o, l, out, NG - 1)
            h = x + jnp.sum(out, axis=0, keepdims=True)
            x1 = _ln(h)
            y = jnp.broadcast_to(_ln(x1).astype(jnp.bfloat16), (8, D))

        G_T0 = SPM * M_T0

        def t_sem(i):
            return sems.at[(G_T0 + i) % (SPM * NM)]

        with scope('T'):
            g = [None] * NF
            acc = None
            for i in range(N_TS):
                a, b = t_step_copies(i, t_sem(i))
                a.wait()
                b.wait()
                if i + NGS < N_TS:
                    a, b = t_step_copies(i + NGS, t_sem(i + NGS))
                    a.start(priority=0)
                    b.start(priority=1)
                d()
                if i % ND == ND - 1:
                    m = (i % 30) // ND
                    for f in (2 * m, 2 * m + 1):
                        if i < 30:
                            g[f] = _gelu(jnp.dot(y, w3b[f], preferred_element_type=jnp.float32)).astype(jnp.bfloat16)
                        else:
                            t = jnp.dot(g[f], w4b[f], preferred_element_type=jnp.float32)
                            acc = t if acc is None else acc + t
            o_ref[0] = (h + (x1 + acc[0:1])).astype(o_ref.dtype)

    @jax.jit
    def run(A_x, A_k_cache, A_v_cache, A_wq, A_wo, B_x, B_w1, B_w2, B_w3, B_w4):
        kT = jnp.swapaxes(A_k_cache, 2, 3).reshape(ROWS, SK)
        vT = jnp.swapaxes(A_v_cache, 2, 3).reshape(ROWS, SK)
        any_spec = pl.BlockSpec(memory_space=pl.ANY)
        return pl.pallas_call(
            kernel,
            out_shape=jax.ShapeDtypeStruct((1, 1, D), jnp.bfloat16),
            in_specs=[any_spec] * 7,
            out_specs=pl.BlockSpec(memory_space=pltpu.VMEM),
            scratch_shapes=[
                pltpu.VMEM((1, D), jnp.bfloat16),
                pltpu.VMEM((2, NCM, GR, CW), jnp.bfloat16),
                pltpu.VMEM((2, NCM, GR, CW), jnp.bfloat16),
                pltpu.VMEM((NG, D, GR), jnp.bfloat16),
                pltpu.VMEM((NG, GR, D), jnp.bfloat16),
                pltpu.VMEM((NF, D, 128), jnp.bfloat16),
                pltpu.VMEM((NF, 128, D), jnp.bfloat16),
                pltpu.VMEM((NCM, 8, CW), jnp.float32),
                pltpu.VMEM((NCM, 8, CW), jnp.bfloat16),
                pltpu.SemaphoreType.DMA,
                pltpu.SemaphoreType.DMA((SPM * NM,)),
                pltpu.SemaphoreType.DMA((NG,)),
                pltpu.SemaphoreType.DMA((NG,)),
            ],
            compiler_params=pltpu.CompilerParams(vmem_limit_bytes=vmem_mb * 1024 * 1024, disable_bounds_checks=True,
                                                 disable_semaphore_checks=nosemchk),
            interpret=interpret,
        )(A_x, kT, vT, A_wq, A_wo, B_w3, B_w4)

    return run


_run = make_kernel(CPM=4, kvc=(32, 512), NGS=36, NM=4)


@jax.jit
def pallas_sequential_preLN__sliding_block_cached__mixer_s_mlp__decode_kernel(
    A_x: jax.Array,
    A_k_cache: jax.Array,
    A_v_cache: jax.Array,
    A_wq: jax.Array,
    A_wo: jax.Array,
    B_x: jax.Array,
    B_w1: jax.Array,
    B_w2: jax.Array,
    B_w3: jax.Array,
    B_w4: jax.Array,
):
    return _run(A_x, A_k_cache, A_v_cache, A_wq, A_wo, B_x, B_w1, B_w2, B_w3, B_w4)
```

```python
import jax
import jax.numpy as jnp
import jax.experimental.pallas as pl
import jax.experimental.pallas.tpu as pltpu

D, H, DH, SK, W, F = 640, 32, 192, 32768, 4096, 1536
ROWS = H * DH
GR = 2 * DH
NG = H // 2
C0 = SK - W
EPS = 1e-5
QG = 4
QW = QG * GR
NQR = D // 8


def _ln(x):
    m = jnp.mean(x, axis=-1, keepdims=True)
    c = x - m
    v = jnp.mean(c * c, axis=-1, keepdims=True)
    return c / jnp.sqrt(v + EPS)


def _gelu(x):
    c = 0.7978845608028654
    return 0.5 * x * (1.0 + jnp.tanh(c * (x + 0.044715 * (x * x * x))))


def make_kernel(CW=512, kvc=(32, 512), NGS=36, NM=4, ro=16, r3=8, r4=24, w4split=(4, 8, 12), xthr=0, q0t=0,
                vmem_mb=64, interpret=False, nocompute=False, scopes=False, wslot0=0):
    NCM = W // CW
    RC, CC = kvc
    NRC, NCC = GR // RC, CW // CC
    SPM = NRC * NCC
    NPM = NCM // 2
    M_S0 = NPM
    M_F0 = M_S0 + (NG - 1) * NCM
    M_T0 = M_F0 + NPM
    LM = -(-NGS // SPM)
    assert SPM * NM >= NGS and NCM & (NCM - 1) == 0 and NM & (NM - 1) == 0 and LM <= NPM
    lg = NCM.bit_length() - 1
    NO = GR // ro
    NQ = NQR // 4
    SPW = NCM * SPM // 32
    assert SPM % SPW == 0 and NO <= 32
    t_stream = [('w3', r) for r in range(0, D, r3)] + [('w4', r) for r in range(0, F, r4)]
    N3 = D // r3
    assert N3 % 2 == 0 and (F // r4) % 2 == 0
    N_TS = len(t_stream) // 2

    class _NoScope:
        def __enter__(self):
            return None

        def __exit__(self, *a):
            return False

    def scope(name):
        return jax.named_scope(name) if scopes else _NoScope()

    def kernel(x_hbm, kT, vT, wq, wo, w3, w4, o_ref,
               xbuf, kbuf, vbuf, wqb, wob, w3b, w4b, s_scr, p_scr, q_scr, xsem, sems, wqsem, wosem):

        def dst_wait(dst, sem):
            pltpu.make_async_copy(dst, dst, sem).wait()

        def when(cond, fn):
            if isinstance(cond, (bool, int)):
                if cond:
                    fn()
            else:
                pl.when(cond)(fn)

        def sem_of(mm, u):
            return sems.at[SPM * (mm & (NM - 1)) + u]

        def kv_dst(buf, pair, cm, u):
            return buf.at[pair & 1, cm, pl.ds((u % NRC) * RC, RC), pl.ds((u // NRC) * CC, CC)]

        def kv_copy(src, buf, pair, cm, u, sem):
            row = pl.multiple_of(pair * GR + (u % NRC) * RC, 8)
            col = pl.multiple_of(C0 + cm * CW + (u // NRC) * CC, 128)
            return pltpu.make_async_copy(src.at[pl.ds(row, RC), pl.ds(col, CC)], kv_dst(buf, pair, cm, u), sem)

        def wq_copy(g, r):
            r0 = pl.multiple_of(r * 8, 8)
            return pltpu.make_async_copy(
                wq.at[pl.ds(r0, 8), pl.ds(pl.multiple_of(g * QW, 128), QW)], wqb.at[g, pl.ds(r0, 8), :], wqsem.at[g])

        def wo_copy(j, i):
            return pltpu.make_async_copy(wo.at[pl.ds(pl.multiple_of(j * GR + i * ro, 8), ro), :],
                                         wob.at[j, pl.ds(pl.multiple_of(i * ro, 8), ro), :], wosem.at[j])

        def t_copy(n, sem):
            kind, r = t_stream[n]
            if kind == 'w3':
                return pltpu.make_async_copy(w3.at[pl.ds(r, r3), :], w3b.at[pl.ds(r, r3), :], sem)
            return pltpu.make_async_copy(w4.at[pl.ds(r, r4), :], w4b.at[pl.ds(r, r4), :], sem)

        def issue_P(m, u):
            sem = sem_of(m, u)
            kv_copy(kT, kbuf, 0, 2 * m, u, sem).start(priority=0)
            kv_copy(kT, kbuf, 0, 2 * m + 1, u, sem).start(priority=1)
            per = -(-NQ // (NPM * SPM))
            for e in range(per):
                i = (m * SPM + u) * per + e
                when(i < NQ, lambda: wq_copy(1, i if isinstance(i, int) else jnp.minimum(i, NQ - 1)).start(priority=1))

        def issue_S(t, u):
            j, cm = t >> lg, t & (NCM - 1)
            sem = sem_of(t + M_S0, u)
            kv_copy(kT, kbuf, j + 1, cm, u, sem).start(priority=0)
            kv_copy(vT, vbuf, j, cm, u, sem).start(priority=1)
            if u % SPW == SPW - 1:
                i = cm * (SPM // SPW) + u // SPW
                jn = j + 1

                @pl.when((i < NQ) & (jn < 3 * QG))
                def _():
                    wq_copy(jnp.minimum(1 + (jn >> 2), 3), (jn & 3) * NQ + jnp.minimum(i, NQ - 1)).start(priority=1)

                @pl.when(i < NO)
                def _():
                    wo_copy(j, jnp.minimum(i, NO - 1)).start(priority=1)

        def issue_F(m, u):
            sem = sem_of(m + M_F0, u)
            kv_copy(vT, vbuf, NG - 1, 2 * m, u, sem).start(priority=0)
            kv_copy(vT, vbuf, NG - 1, 2 * m + 1, u, sem).start(priority=1)
            per = -(-NO // (NPM * SPM))
            for e in range(per):
                i = (m * SPM + u) * per + e
                when(i < NO, lambda: wo_copy(NG - 1, i if isinstance(i, int) else jnp.minimum(i, NO - 1)).start(priority=1))

        def issue_T(m, u):
            for mm in range(LM + 1):
                i = mm * SPM + u
                if i < min(NGS, N_TS):
                    @pl.when(m == mm)
                    def _():
                        sem = sem_of(M_T0 + mm, u)
                        t_copy(2 * i, sem).start(priority=0)
                        t_copy(2 * i + 1, sem).start(priority=1)

        def ahead(m, u):
            return m + (u + NGS) // SPM, (u + NGS) % SPM

        def when_range(mt, lo, hi, fn, u):
            @pl.when((mt >= lo) & (mt < hi))
            def _():
                fn(jnp.clip(mt - lo, 0, hi - lo - 1), u)

        x_copy = pltpu.make_async_copy(x_hbm.at[0], xbuf, xsem)
        x_copy.start(priority=xthr)

        def q0_body(r, _):
            for e in range(4):
                wq_copy(0, 4 * r + e).start(priority=(0 if q0t == 0 else e % 2))
            return 0
        jax.lax.fori_loop(0, NQR // 4, q0_body, 0)

        def pro_body(m, _):
            for u in range(SPM):
                when(m * SPM + u < NGS, lambda: issue_P(m, u))
            return 0
        jax.lax.fori_loop(0, LM, pro_body, 0)

        with scope('xwait'):
            x_copy.wait()
        x = xbuf[...].astype(jnp.float32)
        xn = _ln(x).astype(jnp.bfloat16)
        xn8 = jnp.broadcast_to(xn, (8, D))

        row = jax.lax.broadcasted_iota(jnp.int32, (8, GR), 0)
        col = jax.lax.broadcasted_iota(jnp.int32, (8, GR), 1)
        mask = (col >= row * DH) & (col < (row + 1) * DH)
        scale = DH ** -0.5

        def q_group(g):
            dst_wait(wqb.at[g], wqsem.at[g])
            q = jnp.dot(xn8, wqb[g], preferred_element_type=jnp.float32)
            for i in range(QG):
                q_scr[g * QG + i] = jnp.where(mask, q[:, i * GR:(i + 1) * GR], 0.0).astype(jnp.bfloat16)

        def qk(qa, slot, cm):
            if nocompute:
                return jnp.zeros((8, CW), jnp.float32)
            return jnp.dot(qa, kbuf[slot, cm], preferred_element_type=jnp.float32)

        def pv(slot, cm):
            if nocompute:
                return jnp.zeros((8, GR), jnp.float32)
            return jax.lax.dot_general(p_scr[cm], vbuf[slot, cm], (((1,), (1,)), ((), ())),
                                       preferred_element_type=jnp.float32)

        def softmax():
            s = s_scr[...] * scale
            m = jnp.max(jnp.max(s, axis=0), axis=-1, keepdims=True)
            p = jnp.exp(s - m[None])
            l = jnp.sum(jnp.sum(p, axis=0), axis=-1, keepdims=True)
            p_scr[...] = p.astype(jnp.bfloat16)
            return l

        def out_proj(o, l, out, j):
            o = jnp.where(mask, o / l, 0.0).astype(jnp.bfloat16)
            dst_wait(wob.at[j], wosem.at[j])
            return out + jnp.dot(o, wob[j], preferred_element_type=jnp.float32)

        with scope('q0'):
            q_group(0)

        def p_body(m, _):
            qa = q_scr[0]
            for u in range(SPM):
                sem = sem_of(m, u)
                dst_wait(kv_dst(kbuf, 0, 2 * m, u), sem)
                dst_wait(kv_dst(kbuf, 0, 2 * m + 1, u), sem)
                mt, ut = ahead(m, u)
                when_range(mt, 0, M_S0, issue_P, ut)
                when_range(mt, M_S0, M_F0, issue_S, ut)
            s_scr[2 * m] = qk(qa, 0, 2 * m)
            s_scr[2 * m + 1] = qk(qa, 0, 2 * m + 1)
            return 0

        with scope('P_loop'):
            jax.lax.fori_loop(0, NPM, p_body, 0)
        l0 = softmax()

        def s_iter(j, carry, last):
            out, l = carry
            ks, vs = (j + 1) & 1, j & 1
            qa = q_scr[j + 1]

            def c_body(cm, o):
                t = j * NCM + cm
                mm = M_S0 + t
                for u in range(SPM):
                    sem = sem_of(mm, u)
                    dst_wait(kv_dst(kbuf, ks, cm, u), sem)
                    dst_wait(kv_dst(vbuf, vs, cm, u), sem)
                    if last:
                        mt, ut = ahead(mm, u)
                        when_range(mt, M_S0, M_F0, issue_S, ut)
                        when_range(mt, M_F0, M_T0, issue_F, ut)
                    else:
                        tt, ut = ahead(t, u)
                        issue_S(tt, ut)
                s_scr[cm] = qk(qa, ks, cm)
                return o + pv(vs, cm)

            with scope('S_loop'):
                o = jax.lax.fori_loop(0, NCM, c_body, jnp.zeros((8, GR), jnp.float32))
            out = out_proj(o, l, out, j)
            if not last:
                @pl.when(((j + 2) & 3) == 0)
                def _():
                    q_group(jnp.minimum((j + 2) >> 2, 3))
            return out, softmax()

        out, l = jax.lax.fori_loop(0, NG - 2, lambda j, c: s_iter(j, c, False), (jnp.zeros((8, D), jnp.float32), l0))
        out, l = s_iter(NG - 2, (out, l), True)

        vs = (NG - 1) & 1

        def f_body(m, o):
            mm = M_F0 + m
            for u in range(SPM):
                sem = sem_of(mm, u)
                dst_wait(kv_dst(vbuf, vs, 2 * m, u), sem)
                dst_wait(kv_dst(vbuf, vs, 2 * m + 1, u), sem)
                mt, ut = ahead(mm, u)
                when_range(mt, M_F0, M_T0, issue_F, ut)
                when_range(mt, M_T0, M_T0 + LM + 1, issue_T, ut)
            return o + pv(vs, 2 * m) + pv(vs, 2 * m + 1)

        with scope('F_loop'):
            o = jax.lax.fori_loop(0, NPM, f_body, jnp.zeros((8, GR), jnp.float32))
        with scope('ln1'):
            out = out_proj(o, l, out, NG - 1)
            h = x + jnp.sum(out, axis=0, keepdims=True)
            x1 = _ln(h)
            y = jnp.broadcast_to(_ln(x1).astype(jnp.bfloat16), (8, D))

        G_T0 = SPM * M_T0

        def t_sem(i):
            return sems.at[(G_T0 + i) % (SPM * NM)]

        with scope('T'):
            g = None
            acc = None
            done_rows, splits = 0, [128 * s for s in w4split]
            for i in range(N_TS):
                t_copy(2 * i, t_sem(i)).wait()
                t_copy(2 * i + 1, t_sem(i)).wait()
                if i + NGS < N_TS:
                    t_copy(2 * (i + NGS), t_sem(i + NGS)).start(priority=0)
                    t_copy(2 * (i + NGS) + 1, t_sem(i + NGS)).start(priority=1)
                n_landed = 2 * i + 2
                if g is None and n_landed >= N3:
                    g = _gelu(jnp.dot(y, w3b[...], preferred_element_type=jnp.float32)).astype(jnp.bfloat16)
                rows4 = max(0, n_landed - N3) * r4
                while g is not None and splits and rows4 >= splits[0]:
                    hi = splits.pop(0)
                    t = jnp.dot(g[:, done_rows:hi], w4b[done_rows:hi, :], preferred_element_type=jnp.float32)
                    acc = t if acc is None else acc + t
                    done_rows = hi
            assert done_rows == F and g is not None
            o_ref[0] = (h + (x1 + acc[0:1])).astype(o_ref.dtype)

    @jax.jit
    def run(A_x, A_k_cache, A_v_cache, A_wq, A_wo, B_x, B_w1, B_w2, B_w3, B_w4):
        kT = jnp.swapaxes(A_k_cache, 2, 3).reshape(ROWS, SK)
        vT = jnp.swapaxes(A_v_cache, 2, 3).reshape(ROWS, SK)
        any_spec = pl.BlockSpec(memory_space=pl.ANY)
        return pl.pallas_call(
            kernel,
            out_shape=jax.ShapeDtypeStruct((1, 1, D), jnp.bfloat16),
            in_specs=[any_spec] * 7,
            out_specs=pl.BlockSpec(memory_space=pltpu.VMEM),
            scratch_shapes=[
                pltpu.VMEM((1, D), jnp.bfloat16),
                pltpu.VMEM((2, NCM, GR, CW), jnp.bfloat16),
                pltpu.VMEM((2, NCM, GR, CW), jnp.bfloat16),
                pltpu.VMEM((NG // QG, D, QW), jnp.bfloat16),
                pltpu.VMEM((NG, GR, D), jnp.bfloat16),
                pltpu.VMEM((D, F), jnp.bfloat16),
                pltpu.VMEM((F, D), jnp.bfloat16),
                pltpu.VMEM((NCM, 8, CW), jnp.float32),
                pltpu.VMEM((NCM, 8, CW), jnp.bfloat16),
                pltpu.VMEM((NG, 8, GR), jnp.bfloat16),
                pltpu.SemaphoreType.DMA,
                pltpu.SemaphoreType.DMA((SPM * NM,)),
                pltpu.SemaphoreType.DMA((NG // QG,)),
                pltpu.SemaphoreType.DMA((NG,)),
            ],
            compiler_params=pltpu.CompilerParams(vmem_limit_bytes=vmem_mb * 1024 * 1024, disable_bounds_checks=True,
                                                 disable_semaphore_checks=True),
            interpret=interpret,
        )(A_x, kT, vT, A_wq, A_wo, B_w3, B_w4)

    return run


_run = make_kernel(w4split=(3, 6, 9, 12), q0t=1)


@jax.jit
def pallas_sequential_preLN__sliding_block_cached__mixer_s_mlp__decode_kernel(
    A_x: jax.Array,
    A_k_cache: jax.Array,
    A_v_cache: jax.Array,
    A_wq: jax.Array,
    A_wo: jax.Array,
    B_x: jax.Array,
    B_w1: jax.Array,
    B_w2: jax.Array,
    B_w3: jax.Array,
    B_w4: jax.Array,
):
    return _run(A_x, A_k_cache, A_v_cache, A_wq, A_wo, B_x, B_w1, B_w2, B_w3, B_w4)
```

```python
import jax
import jax.numpy as jnp
import jax.experimental.pallas as pl
import jax.experimental.pallas.tpu as pltpu

D, H, DH, SK, W, F = 640, 32, 192, 32768, 4096, 1536
ROWS = H * DH
GR = 2 * DH
NG = H // 2
C0 = SK - W
EPS = 1e-5

QG = 4
QW = QG * GR
NQR = D // 8
NQ = NQR // 4

CW = 512
RC = 32
NCM = W // CW
SPM = GR // RC
NPM = NCM // 2
M_S0 = NPM
M_F0 = M_S0 + (NG - 1) * NCM
M_T0 = M_F0 + NPM
LG_NCM = NCM.bit_length() - 1

NGS = 38
NM = 4
LM = -(-NGS // SPM)
RO = 16
NO = GR // RO
SPW = NCM * SPM // 32
R3, R4 = 16, 24
W4_SPLITS = (384, 768, 1152, 1536)
V_CSHIFT, V_USHIFT = 0, 2

assert SPM * NM >= NGS and LM <= NPM and NGS <= NQR // 2 and NO <= 32 and SPM % SPW == 0


def _ln(x):
    m = jnp.mean(x, axis=-1, keepdims=True)
    c = x - m
    v = jnp.mean(c * c, axis=-1, keepdims=True)
    return c / jnp.sqrt(v + EPS)


def _gelu(x):
    c = 0.7978845608028654
    return 0.5 * x * (1.0 + jnp.tanh(c * (x + 0.044715 * (x * x * x))))


def _t_stream():
    l3 = [("w3", r) for r in range(0, D, R3)]
    half = len(l3) // 2
    l3 = [c for pair in zip(l3[:half], l3[half:]) for c in pair]
    return l3 + [("w4", r) for r in range(0, F, R4)]


def _kernel(x_hbm, kT, vT, wq, wo, w3, w4, o_ref,
            xbuf, kbuf, vbuf, wqb, wob, w3b, w4b, s_scr, p_scr, q_scr,
            xsem, sems, wqsem, wosem, qsems):
    t_stream = _t_stream()
    n3 = D // R3
    n_ts = len(t_stream) // 2
    nqs = NQR // 2

    def dst_wait(dst, sem):
        pltpu.make_async_copy(dst, dst, sem).wait()

    def when(cond, fn):
        if isinstance(cond, (bool, int)):
            if cond:
                fn()
        else:
            pl.when(cond)(fn)

    def sem_of(mm, u):
        return sems.at[SPM * (mm & (NM - 1)) + u]

    def kv_dst(buf, pair, cm, u):
        return buf.at[pair & 1, cm, pl.ds(u * RC, RC), :]

    def kv_copy(src, buf, pair, cm, u, sem):
        row = pl.multiple_of(pair * GR + u * RC, 8)
        col = pl.multiple_of(C0 + cm * CW, 128)
        return pltpu.make_async_copy(src.at[pl.ds(row, RC), pl.ds(col, CW)], kv_dst(buf, pair, cm, u), sem)

    def wq_copy(g, r, sem):
        r0 = pl.multiple_of(r * 8, 8)
        return pltpu.make_async_copy(
            wq.at[pl.ds(r0, 8), pl.ds(pl.multiple_of(g * QW, 128), QW)], wqb.at[g, pl.ds(r0, 8), :], sem)

    def wo_copy(j, i):
        return pltpu.make_async_copy(wo.at[pl.ds(pl.multiple_of(j * GR + i * RO, 8), RO), :],
                                     wob.at[j, pl.ds(pl.multiple_of(i * RO, 8), RO), :], wosem.at[j])

    def t_copy(n, sem):
        kind, r = t_stream[n]
        if kind == "w3":
            return pltpu.make_async_copy(w3.at[pl.ds(r, R3), :], w3b.at[pl.ds(r, R3), :], sem)
        return pltpu.make_async_copy(w4.at[pl.ds(r, R4), :], w4b.at[pl.ds(r, R4), :], sem)

    def v_cm(cm):
        return (cm + V_CSHIFT) & (NCM - 1)

    def v_u(u):
        return (u + V_USHIFT) % SPM

    def issue_Q(i):
        wq_copy(0, i, qsems.at[i]).start(priority=0)
        wq_copy(0, i + nqs, qsems.at[i]).start(priority=1)

    def issue_P(m, u):
        sem = sem_of(m, u)
        kv_copy(kT, kbuf, 0, m, u, sem).start(priority=0)
        kv_copy(kT, kbuf, 0, m + NPM, u, sem).start(priority=1)
        i = m * SPM + u
        when(i < NQ, lambda: wq_copy(1, i if isinstance(i, int) else jnp.minimum(i, NQ - 1),
                                     wqsem.at[1]).start(priority=1))

    def issue_S(t, u):
        j, cm = t >> LG_NCM, t & (NCM - 1)
        sem = sem_of(t + M_S0, u)
        kv_copy(kT, kbuf, j + 1, cm, u, sem).start(priority=0)
        kv_copy(vT, vbuf, j, v_cm(cm), v_u(u), sem).start(priority=1)
        if u % SPW == SPW - 1:
            i = cm * (SPM // SPW) + u // SPW
            jn = j + 1

            @pl.when((i < NQ) & (jn < 3 * QG))
            def _():
                g = jnp.minimum(1 + (jn >> 2), 3)
                wq_copy(g, (jn & 3) * NQ + jnp.minimum(i, NQ - 1), wqsem.at[g]).start(priority=1)

            @pl.when(i < NO)
            def _():
                wo_copy(j, jnp.minimum(i, NO - 1)).start(priority=1)

    def issue_F(m, u):
        sem = sem_of(m + M_F0, u)
        kv_copy(vT, vbuf, NG - 1, m, u, sem).start(priority=0)
        kv_copy(vT, vbuf, NG - 1, m + NPM, u, sem).start(priority=1)
        i = m * SPM + u
        when(i < NO, lambda: wo_copy(NG - 1, jnp.minimum(i, NO - 1)).start(priority=1))

    def issue_T(m, u):
        for mm in range(LM + 1):
            i = mm * SPM + u
            if i < min(NGS, n_ts):
                @pl.when(m == mm)
                def _():
                    sem = sem_of(M_T0 + mm, u)
                    t_copy(2 * i, sem).start(priority=0)
                    t_copy(2 * i + 1, sem).start(priority=1)

    def ahead(m, u):
        return m + (u + NGS) // SPM, (u + NGS) % SPM

    def when_range(mt, lo, hi, fn, u):
        @pl.when((mt >= lo) & (mt < hi))
        def _():
            fn(jnp.clip(mt - lo, 0, hi - lo - 1), u)

    x_copy = pltpu.make_async_copy(x_hbm.at[0], xbuf, xsem)
    x_copy.start(priority=0)

    def pro_body(i, _):
        issue_Q(i)
        return 0
    jax.lax.fori_loop(0, NGS, pro_body, 0)

    for i in range(nqs):
        wq_copy(0, i, qsems.at[i]).wait()
        wq_copy(0, i + nqs, qsems.at[i]).wait()
        if i + NGS < nqs:
            issue_Q(i + NGS)
        else:
            g = i + NGS - nqs
            issue_P(g // SPM, g % SPM)

    x_copy.wait()
    x = xbuf[...].astype(jnp.float32)
    xn8 = jnp.broadcast_to(_ln(x).astype(jnp.bfloat16), (8, D))

    row = jax.lax.broadcasted_iota(jnp.int32, (8, GR), 0)
    col = jax.lax.broadcasted_iota(jnp.int32, (8, GR), 1)
    mask = (col >= row * DH) & (col < (row + 1) * DH)
    scale = DH ** -0.5

    def q_group(g):
        q = jnp.dot(xn8, wqb[g], preferred_element_type=jnp.float32)
        for i in range(QG):
            q_scr[g * QG + i] = jnp.where(mask, q[:, i * GR:(i + 1) * GR], 0.0).astype(jnp.bfloat16)

    def qk(qa, slot, cm):
        return jnp.dot(qa, kbuf[slot, cm], preferred_element_type=jnp.float32)

    def pv(slot, cm):
        return jax.lax.dot_general(p_scr[cm], vbuf[slot, cm], (((1,), (1,)), ((), ())),
                                   preferred_element_type=jnp.float32)

    def softmax():
        s = s_scr[...] * scale
        m = jnp.max(jnp.max(s, axis=0), axis=-1, keepdims=True)
        p = jnp.exp(s - m[None])
        l = jnp.sum(jnp.sum(p, axis=0), axis=-1, keepdims=True)
        p_scr[...] = p.astype(jnp.bfloat16)
        return l

    def out_proj(o, l, out, j):
        o = jnp.where(mask, o / l, 0.0).astype(jnp.bfloat16)
        dst_wait(wob.at[j], wosem.at[j])
        return out + jnp.dot(o, wob[j], preferred_element_type=jnp.float32)

    q_group(0)

    def p_body(m, _):
        qa = q_scr[0]
        for u in range(SPM):
            sem = sem_of(m, u)
            dst_wait(kv_dst(kbuf, 0, m, u), sem)
            dst_wait(kv_dst(kbuf, 0, m + NPM, u), sem)
            mt, ut = ahead(m, u)
            when_range(mt, 0, M_S0, issue_P, ut)
            when_range(mt, M_S0, M_F0, issue_S, ut)
        s_scr[m] = qk(qa, 0, m)
        s_scr[m + NPM] = qk(qa, 0, m + NPM)
        return 0

    jax.lax.fori_loop(0, NPM, p_body, 0)
    l0 = softmax()

    def s_iter(j, carry, last):
        out, l = carry
        ks, vs = (j + 1) & 1, j & 1
        qa = q_scr[j + 1]

        def c_body(cm, o):
            t = j * NCM + cm
            mm = M_S0 + t
            for u in range(SPM):
                sem = sem_of(mm, u)
                dst_wait(kv_dst(kbuf, ks, cm, u), sem)
                dst_wait(kv_dst(vbuf, vs, v_cm(cm), v_u(u)), sem)
                if last:
                    mt, ut = ahead(mm, u)
                    when_range(mt, M_S0, M_F0, issue_S, ut)
                    when_range(mt, M_F0, M_T0, issue_F, ut)
                else:
                    tt, ut = ahead(t, u)
                    issue_S(tt, ut)
            s_scr[cm] = qk(qa, ks, cm)
            return o + pv(vs, v_cm(cm))

        o = jax.lax.fori_loop(0, NCM, c_body, jnp.zeros((8, GR), jnp.float32))
        out = out_proj(o, l, out, j)
        if not last:
            @pl.when(((j + 2) & 3) == 0)
            def _():
                g = jnp.minimum((j + 2) >> 2, 3)
                dst_wait(wqb.at[g], wqsem.at[g])
                q_group(g)
        return out, softmax()

    out, l = jax.lax.fori_loop(0, NG - 2, lambda j, c: s_iter(j, c, False),
                               (jnp.zeros((8, D), jnp.float32), l0))
    out, l = s_iter(NG - 2, (out, l), True)

    vs = (NG - 1) & 1

    def f_body(m, o):
        mm = M_F0 + m
        for u in range(SPM):
            sem = sem_of(mm, u)
            dst_wait(kv_dst(vbuf, vs, m, u), sem)
            dst_wait(kv_dst(vbuf, vs, m + NPM, u), sem)
            mt, ut = ahead(mm, u)
            when_range(mt, M_F0, M_T0, issue_F, ut)
            when_range(mt, M_T0, M_T0 + LM + 1, issue_T, ut)
        return o + pv(vs, m) + pv(vs, m + NPM)

    o = jax.lax.fori_loop(0, NPM, f_body, jnp.zeros((8, GR), jnp.float32))
    out = out_proj(o, l, out, NG - 1)
    h = x + jnp.sum(out, axis=0, keepdims=True)
    x1 = _ln(h)
    y = jnp.broadcast_to(_ln(x1).astype(jnp.bfloat16), (8, D))

    def t_sem(i):
        return sems.at[(SPM * M_T0 + i) % (SPM * NM)]

    g, acc, done_rows, splits = None, None, 0, list(W4_SPLITS)
    for i in range(n_ts):
        t_copy(2 * i, t_sem(i)).wait()
        t_copy(2 * i + 1, t_sem(i)).wait()
        if i + NGS < n_ts:
            t_copy(2 * (i + NGS), t_sem(i + NGS)).start(priority=0)
            t_copy(2 * (i + NGS) + 1, t_sem(i + NGS)).start(priority=1)
        landed = 2 * i + 2
        if g is None and landed >= n3:
            g = _gelu(jnp.dot(y, w3b[...], preferred_element_type=jnp.float32)).astype(jnp.bfloat16)
        rows4 = max(0, landed - n3) * R4
        while g is not None and splits and rows4 >= splits[0]:
            hi = splits.pop(0)
            t = jnp.dot(g[:, done_rows:hi], w4b[done_rows:hi, :], preferred_element_type=jnp.float32)
            acc = t if acc is None else acc + t
            done_rows = hi
    assert done_rows == F
    o_ref[0] = (h + (x1 + acc[0:1])).astype(o_ref.dtype)


def _call(A_x, A_k_cache, A_v_cache, A_wq, A_wo, B_w3, B_w4, interpret=False):
    kT = jnp.swapaxes(A_k_cache, 2, 3).reshape(ROWS, SK)
    vT = jnp.swapaxes(A_v_cache, 2, 3).reshape(ROWS, SK)
    any_spec = pl.BlockSpec(memory_space=pl.ANY)
    return pl.pallas_call(
        _kernel,
        out_shape=jax.ShapeDtypeStruct((1, 1, D), jnp.bfloat16),
        in_specs=[any_spec] * 7,
        out_specs=pl.BlockSpec(memory_space=pltpu.VMEM),
        scratch_shapes=[
            pltpu.VMEM((1, D), jnp.bfloat16),
            pltpu.VMEM((2, NCM, GR, CW), jnp.bfloat16),
            pltpu.VMEM((2, NCM, GR, CW), jnp.bfloat16),
            pltpu.VMEM((NG // QG, D, QW), jnp.bfloat16),
            pltpu.VMEM((NG, GR, D), jnp.bfloat16),
            pltpu.VMEM((D, F), jnp.bfloat16),
            pltpu.VMEM((F, D), jnp.bfloat16),
            pltpu.VMEM((NCM, 8, CW), jnp.float32),
            pltpu.VMEM((NCM, 8, CW), jnp.bfloat16),
            pltpu.VMEM((NG, 8, GR), jnp.bfloat16),
            pltpu.SemaphoreType.DMA,
            pltpu.SemaphoreType.DMA((SPM * NM,)),
            pltpu.SemaphoreType.DMA((NG // QG,)),
            pltpu.SemaphoreType.DMA((NG,)),
            pltpu.SemaphoreType.DMA((NQR // 2,)),
        ],
        compiler_params=pltpu.CompilerParams(
            vmem_limit_bytes=64 * 1024 * 1024,
            disable_bounds_checks=True,
            disable_semaphore_checks=True,
        ),
        interpret=interpret,
    )(A_x, kT, vT, A_wq, A_wo, B_w3, B_w4)


@jax.jit
def pallas_sequential_preLN__sliding_block_cached__mixer_s_mlp__decode_kernel(
    A_x: jax.Array,
    A_k_cache: jax.Array,
    A_v_cache: jax.Array,
    A_wq: jax.Array,
    A_wo: jax.Array,
    B_x: jax.Array,
    B_w1: jax.Array,
    B_w2: jax.Array,
    B_w3: jax.Array,
    B_w4: jax.Array,
):
    return _call(A_x, A_k_cache, A_v_cache, A_wq, A_wo, B_w3, B_w4)
```

```python
import jax
import jax.numpy as jnp
import jax.experimental.pallas as pl
import jax.experimental.pallas.tpu as pltpu

D, H, DH, SK, W, F = 640, 32, 192, 32768, 4096, 1536
ROWS = H * DH
GR = 2 * DH
NG = H // 2
C0 = SK - W
EPS = 1e-5

QG = 4
QW = QG * GR
NQR = D // 8
NQ = NQR // 4

CW = 512
RC = 32
NCM = W // CW
SPM = GR // RC
NPM = NCM // 2
M_S0 = NPM
M_F0 = M_S0 + (NG - 1) * NCM
M_T0 = M_F0 + NPM
LG_NCM = NCM.bit_length() - 1

NGS = 38
NM = 4
LM = -(-NGS // SPM)
RO = 16
NO = GR // RO
SPW = NCM * SPM // 32
R3, R4 = 16, 24
W4_SPLITS = (384, 768, 1152, 1536)
V_CSHIFT, V_USHIFT = 0, 2

assert SPM * NM >= NGS and LM <= NPM and NGS <= NQR // 2 and NO <= 32 and SPM % SPW == 0


def _ln(x):
    m = jnp.mean(x, axis=-1, keepdims=True)
    c = x - m
    v = jnp.mean(c * c, axis=-1, keepdims=True)
    return c / jnp.sqrt(v + EPS)


def _gelu(x):
    c = 0.7978845608028654
    return 0.5 * x * (1.0 + jnp.tanh(c * (x + 0.044715 * (x * x * x))))


def _t_stream():
    l3 = [("w3", r) for r in range(0, D, R3)]
    half = len(l3) // 2
    l3 = [c for pair in zip(l3[:half], l3[half:]) for c in pair]
    return l3 + [("w4", r) for r in range(0, F, R4)]


def _kernel(x_hbm, kT, vT, wq, wo, w3, w4, o_ref,
            xbuf, kbuf, vbuf, wqb, wob, w3b, w4b, s_scr, p_scr, q_scr,
            xsem, sems, wqsem, wosem, qsems):
    t_stream = _t_stream()
    n3 = D // R3
    n_ts = len(t_stream) // 2
    nqs = NQR // 2

    def total_wait(dst, sem):
        pltpu.make_async_copy(dst, dst, sem).wait()

    def when(cond, fn):
        if isinstance(cond, (bool, int)):
            if cond:
                fn()
        else:
            pl.when(cond)(fn)

    def sem_of(mm, u):
        return sems.at[SPM * (mm & (NM - 1)) + u]

    def kv_dst(buf, pair, cm, u):
        return buf.at[pair & 1, cm, pl.ds(u * RC, RC), :]

    def kv_copy(src, buf, pair, cm, u, sem):
        row = pl.multiple_of(pair * GR + u * RC, 8)
        col = pl.multiple_of(C0 + cm * CW, 128)
        return pltpu.make_async_copy(src.at[pl.ds(row, RC), pl.ds(col, CW)], kv_dst(buf, pair, cm, u), sem)

    def wq_copy(g, r, sem):
        r0 = pl.multiple_of(r * 8, 8)
        return pltpu.make_async_copy(
            wq.at[pl.ds(r0, 8), pl.ds(pl.multiple_of(g * QW, 128), QW)], wqb.at[g, pl.ds(r0, 8), :], sem)

    def wo_copy(j, i):
        return pltpu.make_async_copy(wo.at[pl.ds(pl.multiple_of(j * GR + i * RO, 8), RO), :],
                                     wob.at[j, pl.ds(pl.multiple_of(i * RO, 8), RO), :], wosem.at[j])

    def t_copy(n, sem):
        kind, r = t_stream[n]
        if kind == "w3":
            return pltpu.make_async_copy(w3.at[pl.ds(r, R3), :], w3b.at[pl.ds(r, R3), :], sem)
        return pltpu.make_async_copy(w4.at[pl.ds(r, R4), :], w4b.at[pl.ds(r, R4), :], sem)

    def v_cm(cm):
        return (cm + V_CSHIFT) & (NCM - 1)

    def v_u(u):
        return (u + V_USHIFT) % SPM

    def issue_Q(i):
        wq_copy(0, i, qsems.at[i]).start(priority=0)
        wq_copy(0, i + nqs, qsems.at[i]).start(priority=1)

    def issue_P(m, u):
        sem = sem_of(m, u)
        kv_copy(kT, kbuf, 0, m, u, sem).start(priority=0)
        kv_copy(kT, kbuf, 0, m + NPM, u, sem).start(priority=1)
        i = m * SPM + u
        when(i < NQ, lambda: wq_copy(1, i if isinstance(i, int) else jnp.minimum(i, NQ - 1),
                                     wqsem.at[1]).start(priority=1))

    def issue_S(t, u):
        j, cm = t >> LG_NCM, t & (NCM - 1)
        sem = sem_of(t + M_S0, u)
        kv_copy(kT, kbuf, j + 1, cm, u, sem).start(priority=0)
        kv_copy(vT, vbuf, j, v_cm(cm), v_u(u), sem).start(priority=1)
        if u % SPW == SPW - 1:
            i = cm * (SPM // SPW) + u // SPW
            jn = j + 1

            @pl.when((i < NQ) & (jn < 3 * QG))
            def _():
                g = jnp.minimum(1 + (jn >> 2), 3)
                wq_copy(g, (jn & 3) * NQ + jnp.minimum(i, NQ - 1), wqsem.at[g]).start(priority=1)

            @pl.when(i < NO)
            def _():
                wo_copy(j, jnp.minimum(i, NO - 1)).start(priority=1)

    def issue_F(m, u):
        sem = sem_of(m + M_F0, u)
        kv_copy(vT, vbuf, NG - 1, m, u, sem).start(priority=0)
        kv_copy(vT, vbuf, NG - 1, m + NPM, u, sem).start(priority=1)
        i = m * SPM + u
        when(i < NO, lambda: wo_copy(NG - 1, jnp.minimum(i, NO - 1)).start(priority=1))

    def issue_T(m, u):
        for mm in range(LM + 1):
            i = mm * SPM + u
            if i < min(NGS, n_ts):
                @pl.when(m == mm)
                def _():
                    sem = sem_of(M_T0 + mm, u)
                    t_copy(2 * i, sem).start(priority=0)
                    t_copy(2 * i + 1, sem).start(priority=1)

    def ahead(m, u):
        return m + (u + NGS) // SPM, (u + NGS) % SPM

    def when_range(mt, lo, hi, fn, u):
        @pl.when((mt >= lo) & (mt < hi))
        def _():
            fn(jnp.clip(mt - lo, 0, hi - lo - 1), u)

    x_copy = pltpu.make_async_copy(x_hbm.at[0], xbuf, xsem)
    x_copy.start(priority=0)

    def pro_body(i, _):
        issue_Q(i)
        return 0
    jax.lax.fori_loop(0, NGS, pro_body, 0)

    for i in range(nqs):
        wq_copy(0, i, qsems.at[i]).wait()
        wq_copy(0, i + nqs, qsems.at[i]).wait()
        if i + NGS < nqs:
            issue_Q(i + NGS)
        else:
            g = i + NGS - nqs
            issue_P(g // SPM, g % SPM)

    x_copy.wait()
    x = xbuf[...].astype(jnp.float32)
    xn8 = jnp.broadcast_to(_ln(x).astype(jnp.bfloat16), (8, D))

    row = jax.lax.broadcasted_iota(jnp.int32, (8, GR), 0)
    col = jax.lax.broadcasted_iota(jnp.int32, (8, GR), 1)
    mask = (col >= row * DH) & (col < (row + 1) * DH)
    scale = DH ** -0.5

    def q_group(g):
        q = jnp.dot(xn8, wqb[g], preferred_element_type=jnp.float32)
        for i in range(QG):
            q_scr[g * QG + i] = jnp.where(mask, q[:, i * GR:(i + 1) * GR], 0.0).astype(jnp.bfloat16)

    def qk(qa, slot, cm):
        return jnp.dot(qa, kbuf[slot, cm], preferred_element_type=jnp.float32)

    def pv(slot, cm):
        return jax.lax.dot_general(p_scr[cm], vbuf[slot, cm], (((1,), (1,)), ((), ())),
                                   preferred_element_type=jnp.float32)

    def softmax():
        s = s_scr[...] * scale
        m = jnp.max(jnp.max(s, axis=0), axis=-1, keepdims=True)
        p = jnp.exp(s - m[None])
        l = jnp.sum(jnp.sum(p, axis=0), axis=-1, keepdims=True)
        p_scr[...] = p.astype(jnp.bfloat16)
        return l

    def out_proj(o, l, out, j):
        o = jnp.where(mask, o / l, 0.0).astype(jnp.bfloat16)
        total_wait(wob.at[j], wosem.at[j])
        return out + jnp.dot(o, wob[j], preferred_element_type=jnp.float32)

    q_group(0)

    def p_body(m, _):
        qa = q_scr[0]
        for u in range(SPM):
            sem = sem_of(m, u)
            kv_copy(kT, kbuf, 0, m, u, sem).wait()
            kv_copy(kT, kbuf, 0, m + NPM, u, sem).wait()
            mt, ut = ahead(m, u)
            when_range(mt, 0, M_S0, issue_P, ut)
            when_range(mt, M_S0, M_F0, issue_S, ut)
        s_scr[m] = qk(qa, 0, m)
        s_scr[m + NPM] = qk(qa, 0, m + NPM)
        return 0

    jax.lax.fori_loop(0, NPM, p_body, 0)
    l0 = softmax()

    def s_iter(j, carry, last):
        out, l = carry
        ks, vs = (j + 1) & 1, j & 1
        qa = q_scr[j + 1]

        def c_body(cm, o):
            t = j * NCM + cm
            mm = M_S0 + t
            for u in range(SPM):
                sem = sem_of(mm, u)
                kv_copy(kT, kbuf, j + 1, cm, u, sem).wait()
                kv_copy(vT, vbuf, j, v_cm(cm), v_u(u), sem).wait()
                if last:
                    mt, ut = ahead(mm, u)
                    when_range(mt, M_S0, M_F0, issue_S, ut)
                    when_range(mt, M_F0, M_T0, issue_F, ut)
                else:
                    tt, ut = ahead(t, u)
                    issue_S(tt, ut)
            s_scr[cm] = qk(qa, ks, cm)
            return o + pv(vs, v_cm(cm))

        o = jax.lax.fori_loop(0, NCM, c_body, jnp.zeros((8, GR), jnp.float32))
        out = out_proj(o, l, out, j)
        if not last:
            @pl.when(((j + 2) & 3) == 0)
            def _():
                g = jnp.minimum((j + 2) >> 2, 3)
                total_wait(wqb.at[g], wqsem.at[g])
                q_group(g)
        return out, softmax()

    out, l = jax.lax.fori_loop(0, NG - 2, lambda j, c: s_iter(j, c, False),
                               (jnp.zeros((8, D), jnp.float32), l0))
    out, l = s_iter(NG - 2, (out, l), True)

    vs = (NG - 1) & 1

    def f_body(m, o):
        mm = M_F0 + m
        for u in range(SPM):
            sem = sem_of(mm, u)
            kv_copy(vT, vbuf, NG - 1, m, u, sem).wait()
            kv_copy(vT, vbuf, NG - 1, m + NPM, u, sem).wait()
            mt, ut = ahead(mm, u)
            when_range(mt, M_F0, M_T0, issue_F, ut)
            when_range(mt, M_T0, M_T0 + LM + 1, issue_T, ut)
        return o + pv(vs, m) + pv(vs, m + NPM)

    o = jax.lax.fori_loop(0, NPM, f_body, jnp.zeros((8, GR), jnp.float32))
    out = out_proj(o, l, out, NG - 1)
    h = x + jnp.sum(out, axis=0, keepdims=True)
    x1 = _ln(h)
    y = jnp.broadcast_to(_ln(x1).astype(jnp.bfloat16), (8, D))

    def t_sem(i):
        return sems.at[(SPM * M_T0 + i) % (SPM * NM)]

    g, acc, done_rows, splits = None, None, 0, list(W4_SPLITS)
    for i in range(n_ts):
        t_copy(2 * i, t_sem(i)).wait()
        t_copy(2 * i + 1, t_sem(i)).wait()
        if i + NGS < n_ts:
            t_copy(2 * (i + NGS), t_sem(i + NGS)).start(priority=0)
            t_copy(2 * (i + NGS) + 1, t_sem(i + NGS)).start(priority=1)
        landed = 2 * i + 2
        if g is None and landed >= n3:
            g = _gelu(jnp.dot(y, w3b[...], preferred_element_type=jnp.float32)).astype(jnp.bfloat16)
        rows4 = max(0, landed - n3) * R4
        while g is not None and splits and rows4 >= splits[0]:
            hi = splits.pop(0)
            t = jnp.dot(g[:, done_rows:hi], w4b[done_rows:hi, :], preferred_element_type=jnp.float32)
            acc = t if acc is None else acc + t
            done_rows = hi
    assert done_rows == F
    o_ref[0] = (h + (x1 + acc[0:1])).astype(o_ref.dtype)


def _call(A_x, A_k_cache, A_v_cache, A_wq, A_wo, B_w3, B_w4, interpret=False):
    kT = jnp.swapaxes(A_k_cache, 2, 3).reshape(ROWS, SK)
    vT = jnp.swapaxes(A_v_cache, 2, 3).reshape(ROWS, SK)
    any_spec = pl.BlockSpec(memory_space=pl.ANY)
    return pl.pallas_call(
        _kernel,
        out_shape=jax.ShapeDtypeStruct((1, 1, D), jnp.bfloat16),
        in_specs=[any_spec] * 7,
        out_specs=pl.BlockSpec(memory_space=pltpu.VMEM),
        scratch_shapes=[
            pltpu.VMEM((1, D), jnp.bfloat16),
            pltpu.VMEM((2, NCM, GR, CW), jnp.bfloat16),
            pltpu.VMEM((2, NCM, GR, CW), jnp.bfloat16),
            pltpu.VMEM((NG // QG, D, QW), jnp.bfloat16),
            pltpu.VMEM((NG, GR, D), jnp.bfloat16),
            pltpu.VMEM((D, F), jnp.bfloat16),
            pltpu.VMEM((F, D), jnp.bfloat16),
            pltpu.VMEM((NCM, 8, CW), jnp.float32),
            pltpu.VMEM((NCM, 8, CW), jnp.bfloat16),
            pltpu.VMEM((NG, 8, GR), jnp.bfloat16),
            pltpu.SemaphoreType.DMA,
            pltpu.SemaphoreType.DMA((SPM * NM,)),
            pltpu.SemaphoreType.DMA((NG // QG,)),
            pltpu.SemaphoreType.DMA((NG,)),
            pltpu.SemaphoreType.DMA((NQR // 2,)),
        ],
        compiler_params=pltpu.CompilerParams(
            vmem_limit_bytes=64 * 1024 * 1024,
            disable_bounds_checks=True,
            disable_semaphore_checks=True,
        ),
        interpret=interpret,
    )(A_x, kT, vT, A_wq, A_wo, B_w3, B_w4)


@jax.jit
def pallas_sequential_preLN__sliding_block_cached__mixer_s_mlp__decode_kernel(
    A_x: jax.Array,
    A_k_cache: jax.Array,
    A_v_cache: jax.Array,
    A_wq: jax.Array,
    A_wo: jax.Array,
    B_x: jax.Array,
    B_w1: jax.Array,
    B_w2: jax.Array,
    B_w3: jax.Array,
    B_w4: jax.Array,
):
    return _call(A_x, A_k_cache, A_v_cache, A_wq, A_wo, B_w3, B_w4)
```
